```python
import jax
import jax.numpy as jnp

def _softmax(x, axis=-1):
    return jax.nn.softmax(x, axis=axis)
def _gelu(x):
    return jax.nn.gelu(x, approximate=True)
def _silu(x):
    return jax.nn.silu(x)
def _sigmoid(x):
    return jax.nn.sigmoid(x)
def _layernorm(x, axis=-1, eps=1e-5):
    m = jnp.mean(x, axis=axis, keepdims=True)
    v = jnp.var(x, axis=axis, keepdims=True)
    return (x - m) / jnp.sqrt(v + eps)
def _scatter_add(tgt, idx, src, axis=0):
    return tgt.at[idx].add(src)
def _segment_sum(src, seg, n):
    return jax.ops.segment_sum(src, seg, n)
class _Rng:
    def __init__(self, key):
        self._k = key
    def _next(self):
        self._k, sub = jax.random.split(self._k)
        return sub
    def normal(self, shape):
        return jax.random.normal(self._next(), shape, dtype=jnp.bfloat16)
    def randint(self, lo, hi, shape):
        return jax.random.randint(self._next(), shape, lo, hi, dtype=jnp.int32)
    def uniform(self, shape, lo=0.0, hi=1.0):
        return jax.random.uniform(self._next(), shape, jnp.bfloat16, lo, hi)
    def permutation(self, n):
        return jax.random.permutation(self._next(), n)


kernel_name = 'sequential_preLN__sliding_block_cached__moe_arch_mod__decode'

def setup_inputs():
    _rng = _Rng(jax.random.key(int.from_bytes(__import__("os").urandom(4), "little")))
    _w = (lambda a: (lambda t: t.astype(jnp.bfloat16) if jnp.issubdtype(t.dtype, jnp.floating) else t)(jnp.asarray(a)))
    def _A_setup():
        B, Sq, D = 1, 1, 640
        Hq, Hkv, Sk, Dh = 32, 32, 32768, 192
        assert Hq % Hkv == 0, (Hq, Hkv)
        return {
            "x": _w((lambda *s: _rng.normal(s) * 0.05)(B, Sq, D)),
            "k_cache": _w((lambda *s: _rng.normal(s) * 0.05)(B, Hkv, Sk, Dh)),
            "v_cache": _w((lambda *s: _rng.normal(s) * 0.05)(B, Hkv, Sk, Dh)),
            "wq": _w((lambda *s: _rng.normal(s) * 0.05)(D, Hq * Dh) * (D ** -0.5)),
            "wo": _w((lambda *s: _rng.normal(s) * 0.05)(Hq * Dh, D) * ((Hq * Dh) ** -0.5)),
        }
    _A_in = _A_setup()

    def _B_setup():
        B, S, D, F, C = 1, 1, 640, 1536, 1
        return {
            "x": _w((lambda *s: _rng.normal(s) * 0.05)(B, S, D)),
            "w_r": _w((lambda *s: _rng.normal(s) * 0.05)(D)),
            "w_gate": _w((lambda *s: _rng.normal(s) * 0.05)(D, F)),
            "w_up": _w((lambda *s: _rng.normal(s) * 0.05)(D, F)),
            "w_down": _w((lambda *s: _rng.normal(s) * 0.05)(F, D)),
        }
    _B_in = _B_setup()

    return {
        "A_x": _A_in["x"],
        "A_k_cache": _A_in["k_cache"],
        "A_v_cache": _A_in["v_cache"],
        "A_wq": _A_in["wq"],
        "A_wo": _A_in["wo"],
        "B_x": _B_in["x"],
        "B_w_r": _B_in["w_r"],
        "B_w_gate": _B_in["w_gate"],
        "B_w_up": _B_in["w_up"],
        "B_w_down": _B_in["w_down"],
    }

def reference(A_x, A_k_cache, A_v_cache, A_wq, A_wo, B_x, B_w_r, B_w_gate, B_w_up, B_w_down):
    def _A_ref(x, k_cache, v_cache, wq, wo):
        B, Sq, D = x.shape
        Hq, Dh = 32, 192
        Hkv, Sk = k_cache.shape[1], k_cache.shape[2]
        W = min(4096, max(256, Sk // 4))
        rep = Hq // Hkv
        q = (lambda x, *d: x.transpose(*d))((x @ wq).reshape(B, Sq, Hq, Dh), 0, 2, 1, 3)
        k = jnp.repeat(k_cache[:, :, Sk - W:, :], rep, axis=1)
        v = jnp.repeat(v_cache[:, :, Sk - W:, :], rep, axis=1)
        scores = jnp.einsum("bhqd,bhkd->bhqk", q, k) * (Dh ** -0.5)
        p = _softmax(scores, axis=-1)
        o = jnp.einsum("bhqk,bhkd->bhqd", p, v)
        return (lambda x, *d: x.transpose(*d))(o, 0, 2, 1, 3).reshape(B, Sq, Hq * Dh) @ wo

    def _B_ref(x, w_r, w_gate, w_up, w_down):
        B, S, D = x.shape
        C = 1
        r = x @ w_r
        idx = jnp.argsort(-r, axis=-1)[:, :C]
        idx_e = jnp.repeat(idx.reshape(B, C, 1), D, axis=2)
        x_sel = jnp.take_along_axis(x, idx_e, axis=1)
        g = _silu(x_sel @ w_gate)
        u = x_sel @ w_up
        y = (g * u) @ w_down
        r_sel = _sigmoid(jnp.take_along_axis(r, idx, axis=1))
        y = y * r_sel.reshape(B, C, 1)
        b_off = (jnp.arange(B) * S).reshape(B, 1)
        flat_idx = (idx + b_off).reshape(B * C)
        zero = (x * 0.0).reshape(B * S, D)
        upd = _scatter_add(zero, flat_idx, y.reshape(B * C, D), axis=0)
        return x + upd.reshape(B, S, D)

    x = A_x
    h = x + _A_ref(_layernorm(x, axis=-1), A_k_cache, A_v_cache, A_wq, A_wo)
    h2 = h + _B_ref(_layernorm(h, axis=-1), B_w_r, B_w_gate, B_w_up, B_w_down)
    return h2
```

```python
import functools

import jax
import jax.numpy as jnp
import jax.experimental.pallas as pl
import jax.experimental.pallas.tpu as pltpu

_EPS = 1e-5
_RING = 3
_WD_CHUNKS = 4


def _layernorm(x):
    m = jnp.mean(x, axis=-1, keepdims=True)
    xc = x - m
    v = jnp.mean(xc * xc, axis=-1, keepdims=True)
    return xc / jnp.sqrt(v + _EPS)


def _kernel(x_hbm, k_hbm, v_hbm, wq_hbm, wo_hbm, wr_hbm, wg_hbm, wu_hbm, wd_hbm,
            o_ref,
            x_buf, wr_buf, wq_buf, wo_buf, wg_buf, wu_buf, wd_buf, k_buf, v_buf, q_scr,
            sem_misc, sem_k, sem_v, sem_wo, sem_wd,
            *, H, Dh, W, Sk, D, F):
    R = _RING
    f32, bf16 = jnp.float32, jnp.bfloat16
    wdc = F // _WD_CHUNKS

    def k_copy(h, slot):
        return pltpu.make_async_copy(k_hbm.at[h, :, pl.ds(Sk - W, W)], k_buf.at[slot], sem_k.at[slot])

    def v_copy(h, slot):
        return pltpu.make_async_copy(v_hbm.at[h, :, pl.ds(Sk - W, W)], v_buf.at[slot], sem_v.at[slot])

    def wo_copy(h, slot):
        rows = pl.ds(pl.multiple_of(h * Dh, Dh), Dh)
        return pltpu.make_async_copy(wo_hbm.at[rows, :], wo_buf.at[slot], sem_wo.at[slot])

    wq_copy = pltpu.make_async_copy(wq_hbm, wq_buf, sem_misc.at[0])
    x_copy = pltpu.make_async_copy(x_hbm, x_buf, sem_misc.at[1])
    wr_copy = pltpu.make_async_copy(wr_hbm, wr_buf, sem_misc.at[2])
    wg_copy = pltpu.make_async_copy(wg_hbm, wg_buf, sem_misc.at[3])
    wu_copy = pltpu.make_async_copy(wu_hbm, wu_buf, sem_misc.at[4])
    wd_copies = [
        pltpu.make_async_copy(wd_hbm.at[pl.ds(c * wdc, wdc), :], wd_buf.at[pl.ds(c * wdc, wdc), :], sem_wd.at[c])
        for c in range(_WD_CHUNKS)
    ]

    wq_copy.start()
    x_copy.start()
    wr_copy.start()
    for h in range(R):
        k_copy(h, h).start()
        v_copy(h, h).start()
        wo_copy(h, h).start()

    x_copy.wait()
    x = x_buf[...].astype(f32)
    xn = jnp.broadcast_to(_layernorm(x), (8, D)).astype(bf16)
    wq_copy.wait()
    q_all = jnp.dot(xn, wq_buf[...], preferred_element_type=f32)
    for h in range(H):
        q_scr[h] = q_all[:, h * Dh:(h + 1) * Dh].astype(bf16)

    scale = Dh ** -0.5

    def head(h, acc):
        slot = h % R
        k_copy(h, slot).wait()
        s = jnp.dot(q_scr[h], k_buf[slot], preferred_element_type=f32) * scale

        @pl.when(h + R < H)
        def _():
            k_copy(h + R, slot).start()

        m = jnp.max(s, axis=-1, keepdims=True)
        p = jnp.exp(s - m)
        l = jnp.sum(p, axis=-1, keepdims=True)
        v_copy(h, slot).wait()
        o = jax.lax.dot_general(p.astype(bf16), v_buf[slot], (((1,), (1,)), ((), ())),
                                preferred_element_type=f32)
        o = (o / l).astype(bf16)
        wo_copy(h, slot).wait()
        acc = acc + jnp.dot(o, wo_buf[slot], preferred_element_type=f32)

        @pl.when(h + R < H)
        def _():
            v_copy(h + R, slot).start()
            wo_copy(h + R, slot).start()

        @pl.when(h + R == H)
        def _():
            wg_copy.start()
            wu_copy.start()
            for c in wd_copies:
                c.start()

        return acc

    attn = jax.lax.fori_loop(0, H, head, jnp.zeros((8, D), f32))

    hres = x + attn
    hn = _layernorm(hres)
    hn_b = hn.astype(bf16)
    wr_copy.wait()
    wr = wr_buf[...].astype(f32)
    r = jnp.zeros((8, 1), f32)
    for i in range(D // 128):
        r = r + jnp.sum(hn[:, i * 128:(i + 1) * 128] * wr[i:i + 1, :], axis=-1, keepdims=True)
    gate = jax.nn.sigmoid(r)
    wg_copy.wait()
    g = jnp.dot(hn_b, wg_buf[...], preferred_element_type=f32)
    g = g * jax.nn.sigmoid(g)
    wu_copy.wait()
    u = jnp.dot(hn_b, wu_buf[...], preferred_element_type=f32)
    a = (g * u).astype(bf16)
    y = jnp.zeros((8, D), f32)
    for c in range(_WD_CHUNKS):
        wd_copies[c].wait()
        y = y + jnp.dot(a[:, c * wdc:(c + 1) * wdc], wd_buf[pl.ds(c * wdc, wdc), :],
                        preferred_element_type=f32)
    out = hres + hn + y * gate
    o_ref[...] = out[0:1, :].astype(o_ref.dtype)


@jax.jit
def pallas_sequential_preLN__sliding_block_cached__moe_arch_mod__decode_kernel(
    A_x: jax.Array,
    A_k_cache: jax.Array,
    A_v_cache: jax.Array,
    A_wq: jax.Array,
    A_wo: jax.Array,
    B_x: jax.Array,
    B_w_r: jax.Array,
    B_w_gate: jax.Array,
    B_w_up: jax.Array,
    B_w_down: jax.Array,
):
    B, Sq, D = A_x.shape
    _, H, Sk, Dh = A_k_cache.shape
    F = B_w_gate.shape[1]
    W = min(4096, max(256, Sk // 4))
    assert B == 1 and Sq == 1 and A_wq.shape == (D, H * Dh)
    bf16 = jnp.bfloat16

    kT = jnp.swapaxes(A_k_cache, 2, 3).reshape(H, Dh, Sk)
    vT = jnp.swapaxes(A_v_cache, 2, 3).reshape(H, Dh, Sk)

    any_spec = pl.BlockSpec(memory_space=pl.ANY)
    out = pl.pallas_call(
        functools.partial(_kernel, H=H, Dh=Dh, W=W, Sk=Sk, D=D, F=F),
        out_shape=jax.ShapeDtypeStruct((1, D), bf16),
        in_specs=[any_spec] * 9,
        out_specs=pl.BlockSpec(memory_space=pltpu.VMEM),
        scratch_shapes=[
            pltpu.VMEM((1, D), bf16),
            pltpu.VMEM((D // 128, 128), bf16),
            pltpu.VMEM((D, H * Dh), bf16),
            pltpu.VMEM((_RING, Dh, D), bf16),
            pltpu.VMEM((D, F), bf16),
            pltpu.VMEM((D, F), bf16),
            pltpu.VMEM((F, D), bf16),
            pltpu.VMEM((_RING, Dh, W), bf16),
            pltpu.VMEM((_RING, Dh, W), bf16),
            pltpu.VMEM((H, 8, Dh), bf16),
            pltpu.SemaphoreType.DMA((5,)),
            pltpu.SemaphoreType.DMA((_RING,)),
            pltpu.SemaphoreType.DMA((_RING,)),
            pltpu.SemaphoreType.DMA((_RING,)),
            pltpu.SemaphoreType.DMA((_WD_CHUNKS,)),
        ],
        compiler_params=pltpu.CompilerParams(vmem_limit_bytes=64 * 1024 * 1024),
    )(A_x.reshape(1, D), kT, vT, A_wq, A_wo, B_w_r.reshape(D // 128, 128), B_w_gate, B_w_up, B_w_down)
    return out.reshape(B, Sq, D)
```

```python
import functools

import jax
import jax.numpy as jnp
import jax.experimental.pallas as pl
import jax.experimental.pallas.tpu as pltpu

_EPS = 1e-5

_CFG = dict(
    kv_blk=(96, 128), kv_asg="alt",
    wq_blk=(80, 128), wq_asg="alt",
    wo_blk=(32, 640), wo_asg="alt",
    wgu_blk=(80, 128), wgu_asg="alt",
    wd_blk=(32, 640), wd_asg="alt",
    wd_rows=(384, 384, 384, 384),
    mix=True,
    mix_ffn=False,
)


def _layernorm(x):
    m = jnp.mean(x, axis=-1, keepdims=True)
    xc = x - m
    v = jnp.mean(xc * xc, axis=-1, keepdims=True)
    return xc / jnp.sqrt(v + _EPS)


def _blocks(src, dst, sem, blk, asg="alt", order="r"):
    rows, cols = dst.shape
    br, bc = blk
    assert rows % br == 0 and cols % bc == 0, (dst.shape, blk)
    nr, nc = rows // br, cols // bc
    if order == "r":
        allb = [(r, c) for c in range(nc) for r in range(nr)]
    else:
        allb = [(r, c) for r in range(nr) for c in range(nc)]
    if asg == "alt":
        t0, t1 = allb[0::2], allb[1::2]
    elif asg == "rowhalf":
        t0 = [b for b in allb if b[0] < nr // 2]
        t1 = [b for b in allb if b[0] >= nr // 2]
    elif asg == "colhalf":
        t0 = [b for b in allb if b[1] < nc // 2]
        t1 = [b for b in allb if b[1] >= nc // 2]
    seq = []
    for i in range(max(len(t0), len(t1))):
        if i < len(t0):
            seq.append((t0[i], 0))
        if i < len(t1):
            seq.append((t1[i], 1))
    assert len(seq) == len(allb)
    out = []
    for (r, c), p in seq:
        idx = (pl.ds(r * br, br), pl.ds(c * bc, bc))
        out.append((src.at[idx], dst.at[idx], sem, p))
    return out


def _merge(main, extra):
    if not extra:
        return list(main)
    out = []
    n, m = len(main), len(extra)
    k = 0
    for i, d in enumerate(main):
        out.append(d)
        while k < m and (k + 1) * n <= (i + 1) * (m + 1) - 0 and k < m and (i + 1) * (m + 1) >= (k + 1) * n:
            out.append(extra[k])
            k += 1
    out.extend(extra[k:])
    return out


def _issue(descs):
    for src, dst, sem, p in descs:
        pltpu.make_async_copy(src, dst, sem).start(priority=p)


def _wait_all(dst, sem):
    pltpu.make_async_copy(dst, dst, sem).wait()


def _kernel(x_hbm, k_hbm, v_hbm, wq_hbm, wo_hbm, wr_hbm, wg_hbm, wu_hbm, wd_hbm,
            o_ref,
            x_buf, wr_buf, wq_buf, wo_buf, wg_buf, wu_buf, wd_buf, k_buf, v_buf,
            sem_misc, sem_wq, sem_k, sem_v, sem_wo, sem_wd,
            *, H, Dh, W, Sk, D, F, cfg):
    f32, bf16 = jnp.float32, jnp.bfloat16
    wd_rows = cfg["wd_rows"]
    assert sum(wd_rows) == F
    wd_off = [sum(wd_rows[:i]) for i in range(len(wd_rows))]
    NP = H // 2
    nocompute = cfg.get("nocompute")
    mix = cfg["mix"]
    mix_ffn = cfg["mix_ffn"]

    def k_descs(h, slot):
        return _blocks(k_hbm.at[h, :, pl.ds(Sk - W, W)], k_buf.at[slot], sem_k.at[slot], cfg["kv_blk"], cfg["kv_asg"])

    def v_descs(h, slot):
        return _blocks(v_hbm.at[h, :, pl.ds(Sk - W, W)], v_buf.at[slot], sem_v.at[slot], cfg["kv_blk"], cfg["kv_asg"])

    def wo_descs(h, slot):
        rows = pl.ds(pl.multiple_of(h * Dh, Dh), Dh)
        return _blocks(wo_hbm.at[rows, :], wo_buf.at[slot], sem_wo.at[slot], cfg["wo_blk"], cfg["wo_asg"])

    def wq_descs(j, slot):
        cols = pl.ds(pl.multiple_of(j * (2 * Dh), 2 * Dh), 2 * Dh)
        return _blocks(wq_hbm.at[:, cols], wq_buf.at[slot], sem_wq.at[slot], cfg["wq_blk"], cfg["wq_asg"])

    wg_descs = _blocks(wg_hbm, wg_buf, sem_misc.at[2], cfg["wgu_blk"], cfg["wgu_asg"])
    wu_descs = _blocks(wu_hbm, wu_buf, sem_misc.at[3], cfg["wgu_blk"], cfg["wgu_asg"])
    wd_descs = []
    for c, (o, n) in enumerate(zip(wd_off, wd_rows)):
        rows = pl.ds(o, n)
        wd_descs += _blocks(wd_hbm.at[rows, :], wd_buf.at[rows, :], sem_wd.at[c], cfg["wd_blk"], cfg["wd_asg"])

    def comb(main, extra):
        return _merge(main, extra) if mix else list(extra) + list(main)

    x_copy = pltpu.make_async_copy(x_hbm, x_buf, sem_misc.at[0])
    wr_copy = pltpu.make_async_copy(wr_hbm, wr_buf, sem_misc.at[1])

    x_copy.start()
    _issue(wq_descs(0, 0))
    _issue(k_descs(0, 0))
    wr_copy.start()
    x_copy.wait()
    x = x_buf[...].astype(f32)
    xn = jnp.broadcast_to(_layernorm(x), (8, D)).astype(bf16)
    _issue(comb(v_descs(0, 0), wo_descs(0, 0)))
    _issue(k_descs(1, 1))
    _issue(comb(v_descs(1, 1), wo_descs(1, 1)))

    scale = Dh ** -0.5

    def head(q, slot, acc, after_qk, after_pv):
        _wait_all(k_buf.at[slot], sem_k.at[slot])
        if nocompute:
            s = jnp.broadcast_to(q[:, 0:1].astype(f32), (8, 128))
        else:
            s = jnp.dot(q, k_buf[slot], preferred_element_type=f32) * scale
        after_qk()
        m = jnp.max(s, axis=-1, keepdims=True)
        p = jnp.exp(s - m)
        l = jnp.sum(p, axis=-1, keepdims=True)
        _wait_all(v_buf.at[slot], sem_v.at[slot])
        if nocompute:
            o = jnp.broadcast_to(p[:, 0:1], (8, Dh))
        else:
            o = jax.lax.dot_general(p.astype(bf16), v_buf[slot], (((1,), (1,)), ((), ())),
                                    preferred_element_type=f32)
        o = (o / l).astype(bf16)
        _wait_all(wo_buf.at[slot], sem_wo.at[slot])
        acc = acc + jnp.dot(o, wo_buf[slot], preferred_element_type=f32)
        after_pv()
        return acc

    hg, hu = len(wg_descs) // 2, len(wu_descs) // 2

    def pair(j, acc, mode):
        wslot = j % 2
        _wait_all(wq_buf.at[wslot], sem_wq.at[wslot])
        q2 = jnp.dot(xn, wq_buf[wslot], preferred_element_type=f32)
        qa = q2[:, :Dh].astype(bf16)
        qb = q2[:, Dh:].astype(bf16)
        if mode != "last":
            nxt = 2 * j + 2
            ex = [[], [], [], []]
            if mode == "penult":
                ex = [wg_descs[:hg], wg_descs[hg:], wu_descs[:hu], wu_descs[hu:]]
            acc = head(qa, 0, acc,
                       lambda: _issue(comb(k_descs(nxt, 0), wq_descs(j + 1, 1 - wslot) + ex[0])),
                       lambda: _issue(comb(v_descs(nxt, 0), wo_descs(nxt, 0) + ex[1])))
            acc = head(qb, 1, acc,
                       lambda: _issue(comb(k_descs(nxt + 1, 1), ex[2])),
                       lambda: _issue(comb(v_descs(nxt + 1, 1), wo_descs(nxt + 1, 1) + ex[3])))
        elif mix_ffn:
            acc = head(qa, 0, acc, lambda: None, lambda: None)
            acc = head(qb, 1, acc, lambda: _issue(wd_descs), lambda: None)
        else:
            acc = head(qa, 0, acc, lambda: _issue(wg_descs), lambda: None)
            acc = head(qb, 1, acc, lambda: _issue(wu_descs), lambda: None)
        return acc

    n_main = NP - 2 if mix_ffn else NP - 1
    acc = jax.lax.fori_loop(0, n_main, lambda j, a: pair(j, a, "main"), jnp.zeros((8, D), f32))
    if mix_ffn:
        acc = pair(NP - 2, acc, "penult")
    attn = pair(NP - 1, acc, "last")

    hres = x + attn
    hn = _layernorm(hres)
    hn_b = hn.astype(bf16)
    wr_copy.wait()
    wr = wr_buf[...].astype(f32)
    r = jnp.zeros((8, 1), f32)
    for i in range(D // 128):
        r = r + jnp.sum(hn[:, i * 128:(i + 1) * 128] * wr[i:i + 1, :], axis=-1, keepdims=True)
    gate = jax.nn.sigmoid(r)
    base = hres + hn
    if not mix_ffn:
        _issue(wd_descs)
    _wait_all(wg_buf, sem_misc.at[2])
    g = jnp.dot(hn_b, wg_buf[...], preferred_element_type=f32)
    g = g * jax.nn.sigmoid(g)
    _wait_all(wu_buf, sem_misc.at[3])
    u = jnp.dot(hn_b, wu_buf[...], preferred_element_type=f32)
    a = (g * u).astype(bf16)
    y = jnp.zeros((8, D), f32)
    for c, (o, n) in enumerate(zip(wd_off, wd_rows)):
        rows = pl.ds(o, n)
        _wait_all(wd_buf.at[rows, :], sem_wd.at[c])
        y = y + jnp.dot(a[:, o:o + n], wd_buf[rows, :], preferred_element_type=f32)
    out = base + y * gate
    o_ref[...] = out[0:1, :].astype(o_ref.dtype)


def _forward(A_x, A_k_cache, A_v_cache, A_wq, A_wo, B_w_r, B_w_gate, B_w_up, B_w_down, cfg):
    B, Sq, D = A_x.shape
    _, H, Sk, Dh = A_k_cache.shape
    F = B_w_gate.shape[1]
    W = min(4096, max(256, Sk // 4))
    assert B == 1 and Sq == 1 and A_wq.shape == (D, H * Dh) and H % 2 == 0
    bf16 = jnp.bfloat16

    kT = jnp.swapaxes(A_k_cache, 2, 3).reshape(H, Dh, Sk)
    vT = jnp.swapaxes(A_v_cache, 2, 3).reshape(H, Dh, Sk)

    any_spec = pl.BlockSpec(memory_space=pl.ANY)
    out = pl.pallas_call(
        functools.partial(_kernel, H=H, Dh=Dh, W=W, Sk=Sk, D=D, F=F, cfg=cfg),
        out_shape=jax.ShapeDtypeStruct((1, D), bf16),
        in_specs=[any_spec] * 9,
        out_specs=pl.BlockSpec(memory_space=pltpu.VMEM),
        scratch_shapes=[
            pltpu.VMEM((1, D), bf16),
            pltpu.VMEM((D // 128, 128), bf16),
            pltpu.VMEM((2, D, 2 * Dh), bf16),
            pltpu.VMEM((2, Dh, D), bf16),
            pltpu.VMEM((D, F), bf16),
            pltpu.VMEM((D, F), bf16),
            pltpu.VMEM((F, D), bf16),
            pltpu.VMEM((2, Dh, W), bf16),
            pltpu.VMEM((2, Dh, W), bf16),
            pltpu.SemaphoreType.DMA((4,)),
            pltpu.SemaphoreType.DMA((2,)),
            pltpu.SemaphoreType.DMA((2,)),
            pltpu.SemaphoreType.DMA((2,)),
            pltpu.SemaphoreType.DMA((2,)),
            pltpu.SemaphoreType.DMA((len(cfg["wd_rows"]),)),
        ],
        compiler_params=pltpu.CompilerParams(vmem_limit_bytes=64 * 1024 * 1024,
                                             disable_bounds_checks=True),
    )(A_x.reshape(1, D), kT, vT, A_wq, A_wo, B_w_r.reshape(D // 128, 128), B_w_gate, B_w_up, B_w_down)
    return out.reshape(B, Sq, D)


@jax.jit
def pallas_sequential_preLN__sliding_block_cached__moe_arch_mod__decode_kernel(
    A_x: jax.Array,
    A_k_cache: jax.Array,
    A_v_cache: jax.Array,
    A_wq: jax.Array,
    A_wo: jax.Array,
    B_x: jax.Array,
    B_w_r: jax.Array,
    B_w_gate: jax.Array,
    B_w_up: jax.Array,
    B_w_down: jax.Array,
):
    return _forward(A_x, A_k_cache, A_v_cache, A_wq, A_wo, B_w_r, B_w_gate, B_w_up, B_w_down, _CFG)
```

```python
import contextlib
import functools

import jax
import jax.numpy as jnp
import jax.experimental.pallas as pl
import jax.experimental.pallas.tpu as pltpu

_EPS = 1e-5

_CFG = dict(
    kv_blk=(96, 128),
    wq_blk=(80, 128),
    wo_blk=(32, 640),
    wgu_blk=(160, 128),
    wd_blk=(32, 640),
    wd_rows=(512, 512, 256, 128, 128),
    wd_asg=("alt", "alt", "t1", "t1", "t1"),
)


def _layernorm(x):
    m = jnp.mean(x, axis=-1, keepdims=True)
    xc = x - m
    v = jnp.mean(xc * xc, axis=-1, keepdims=True)
    return xc / jnp.sqrt(v + _EPS)


def _blocks(src, dst, sem, blk, asg="alt"):
    rows, cols = dst.shape
    br, bc = blk
    assert rows % br == 0 and cols % bc == 0, (dst.shape, blk)
    out = []
    for c in range(cols // bc):
        for r in range(rows // br):
            idx = (pl.ds(r * br, br), pl.ds(c * bc, bc))
            thread = {"alt": len(out) % 2, "t0": 0, "t1": 1}[asg]
            out.append((src.at[idx], dst.at[idx], sem, thread))
    return out


def _merge(main, extra):
    out, k = [], 0
    n, m = len(main), len(extra)
    for i, d in enumerate(main):
        out.append(d)
        while k < m and (i + 1) * (m + 1) >= (k + 1) * n:
            out.append(extra[k])
            k += 1
    out.extend(extra[k:])
    return out


def _issue(descs):
    for src, dst, sem, thread in descs:
        pltpu.make_async_copy(src, dst, sem).start(priority=thread)


def _kernel(x_hbm, k_hbm, v_hbm, wq_hbm, wo_hbm, wr_hbm, wg_hbm, wu_hbm, wd_hbm,
            o_ref,
            x_buf, wr_buf, wq_buf, wo_buf, wg_buf, wu_buf, wd_buf, k_buf, v_buf,
            sem_misc, sem_k, sem_v, sem_wd,
            *, H, Dh, W, Sk, D, F, cfg):
    f32, bf16 = jnp.float32, jnp.bfloat16
    wd_rows = cfg["wd_rows"]
    assert sum(wd_rows) == F
    wd_off = [sum(wd_rows[:i]) for i in range(len(wd_rows))]
    NP = H // 2
    win = pl.ds(Sk - W, W)
    scopes = cfg.get("scopes")

    def scope(name):
        return jax.named_scope(name) if (scopes and name) else contextlib.nullcontext()

    def wait_all(sem, *dsts):
        for dst in dsts:
            pltpu.make_async_copy(dst, dst, sem).wait()

    def k_descs(h, slot, wq_slot=None):
        sem = sem_k.at[slot]
        kd = _blocks(k_hbm.at[h, :, win], k_buf.at[slot], sem, cfg["kv_blk"])
        if wq_slot is None:
            return kd
        cols = pl.ds(pl.multiple_of(h * Dh, 2 * Dh), 2 * Dh)
        return _merge(kd, _blocks(wq_hbm.at[:, cols], wq_buf.at[wq_slot], sem, cfg["wq_blk"]))

    def v_descs(h, slot):
        sem = sem_v.at[slot]
        vd = _blocks(v_hbm.at[h, :, win], v_buf.at[slot], sem, cfg["kv_blk"])
        rows = pl.ds(pl.multiple_of(h * Dh, Dh), Dh)
        return _merge(vd, _blocks(wo_hbm.at[rows, :], wo_buf.at[slot], sem, cfg["wo_blk"]))

    wg_descs = _blocks(wg_hbm, wg_buf, sem_misc.at[2], cfg["wgu_blk"])
    wu_descs = _blocks(wu_hbm, wu_buf, sem_misc.at[3], cfg["wgu_blk"])
    wd_descs = []
    for c, (o, n) in enumerate(zip(wd_off, wd_rows)):
        rows = pl.ds(o, n)
        blk = cfg["wd_blk"] if n % cfg["wd_blk"][0] == 0 else (n, D)
        asg = cfg["wd_asg"] if isinstance(cfg["wd_asg"], str) else cfg["wd_asg"][c]
        wd_descs += _blocks(wd_hbm.at[rows, :], wd_buf.at[rows, :], sem_wd.at[c], blk, asg)

    x_copy = pltpu.make_async_copy(x_hbm, x_buf, sem_misc.at[0])
    wr_copy = pltpu.make_async_copy(wr_hbm, wr_buf, sem_misc.at[1])

    x_copy.start()
    wr_copy.start()
    _issue(k_descs(0, 0, 0))
    x_copy.wait()
    x = x_buf[...].astype(f32)
    xn = jnp.broadcast_to(_layernorm(x), (8, D)).astype(bf16)
    _issue(v_descs(0, 0))
    _issue(k_descs(1, 1))
    _issue(v_descs(1, 1))

    scale = Dh ** -0.5

    def head(q, slot, acc, after_qk, after_pv, tag=None):
        s = jnp.dot(q, k_buf[slot], preferred_element_type=f32) * scale
        with scope(tag and tag + "_issue1"):
            after_qk()
        m = jnp.max(s, axis=-1, keepdims=True)
        p = jnp.exp(s - m)
        l = jnp.sum(p, axis=-1, keepdims=True)
        with scope(tag and tag + "_vwait"):
            wait_all(sem_v.at[slot], v_buf.at[slot], wo_buf.at[slot])
        o = jax.lax.dot_general(p.astype(bf16), v_buf[slot], (((1,), (1,)), ((), ())),
                                preferred_element_type=f32)
        o = (o / l).astype(bf16)
        acc = acc + jnp.dot(o, wo_buf[slot], preferred_element_type=f32)
        after_pv()
        return acc

    def pair(j, acc, last):
        wslot = j % 2
        wait_all(sem_k.at[0], k_buf.at[0], wq_buf.at[wslot])
        q2 = jnp.dot(xn, wq_buf[wslot], preferred_element_type=f32)
        qa = q2[:, :Dh].astype(bf16)
        qb = q2[:, Dh:].astype(bf16)
        nxt = 2 * j + 2
        nop = lambda: None
        if not last:
            acc = head(qa, 0, acc, lambda: _issue(k_descs(nxt, 0, 1 - wslot)), lambda: _issue(v_descs(nxt, 0)))
            wait_all(sem_k.at[1], k_buf.at[1])
            acc = head(qb, 1, acc, lambda: _issue(k_descs(nxt + 1, 1)), lambda: _issue(v_descs(nxt + 1, 1)))
        else:
            acc = head(qa, 0, acc, lambda: _issue(wg_descs), nop, "h30")
            with scope("h31_kwait"):
                wait_all(sem_k.at[1], k_buf.at[1])
            acc = head(qb, 1, acc, lambda: _issue(wu_descs), nop, "h31")
        return acc

    def main_pair(j, a):
        with scope("pair"):
            return pair(j, a, False)

    acc = jax.lax.fori_loop(0, NP - 1, main_pair, jnp.zeros((8, D), f32))
    with scope("lastpair"):
        attn = pair(NP - 1, acc, True)

    hres = x + attn
    hn = _layernorm(hres)
    hn_b = hn.astype(bf16)
    wr_copy.wait()
    wr = wr_buf[...].astype(f32)
    r = jnp.zeros((8, 1), f32)
    for i in range(D // 128):
        r = r + jnp.sum(hn[:, i * 128:(i + 1) * 128] * wr[i:i + 1, :], axis=-1, keepdims=True)
    gate = jax.nn.sigmoid(r)
    base = hres + hn
    with scope("wd_issue"):
        _issue(wd_descs)
    with scope("wg_wait"):
        wait_all(sem_misc.at[2], wg_buf)
    g = jnp.dot(hn_b, wg_buf[...], preferred_element_type=f32)
    g = g * jax.nn.sigmoid(g)
    with scope("wu_wait"):
        wait_all(sem_misc.at[3], wu_buf)
    u = jnp.dot(hn_b, wu_buf[...], preferred_element_type=f32)
    a = (g * u).astype(bf16)
    y = jnp.zeros((8, D), f32)
    for c, (o, n) in enumerate(zip(wd_off, wd_rows)):
        rows = pl.ds(o, n)
        with scope(f"wd_wait{c}"):
            wait_all(sem_wd.at[c], wd_buf.at[rows, :])
        y = y + jnp.dot(a[:, o:o + n], wd_buf[rows, :], preferred_element_type=f32)
    out = base + y * gate
    o_ref[...] = out[0:1, :].astype(o_ref.dtype)


def _forward(A_x, A_k_cache, A_v_cache, A_wq, A_wo, B_w_r, B_w_gate, B_w_up, B_w_down, cfg):
    B, Sq, D = A_x.shape
    _, H, Sk, Dh = A_k_cache.shape
    F = B_w_gate.shape[1]
    W = min(4096, max(256, Sk // 4))
    assert B == 1 and Sq == 1 and A_wq.shape == (D, H * Dh) and H % 2 == 0
    bf16 = jnp.bfloat16

    kT = jnp.swapaxes(A_k_cache, 2, 3).reshape(H, Dh, Sk)
    vT = jnp.swapaxes(A_v_cache, 2, 3).reshape(H, Dh, Sk)

    any_spec = pl.BlockSpec(memory_space=pl.ANY)
    out = pl.pallas_call(
        functools.partial(_kernel, H=H, Dh=Dh, W=W, Sk=Sk, D=D, F=F, cfg=cfg),
        out_shape=jax.ShapeDtypeStruct((1, D), bf16),
        in_specs=[any_spec] * 9,
        out_specs=pl.BlockSpec(memory_space=pltpu.VMEM),
        scratch_shapes=[
            pltpu.VMEM((1, D), bf16),
            pltpu.VMEM((D // 128, 128), bf16),
            pltpu.VMEM((2, D, 2 * Dh), bf16),
            pltpu.VMEM((2, Dh, D), bf16),
            pltpu.VMEM((D, F), bf16),
            pltpu.VMEM((D, F), bf16),
            pltpu.VMEM((F, D), bf16),
            pltpu.VMEM((2, Dh, W), bf16),
            pltpu.VMEM((2, Dh, W), bf16),
            pltpu.SemaphoreType.DMA((4,)),
            pltpu.SemaphoreType.DMA((2,)),
            pltpu.SemaphoreType.DMA((2,)),
            pltpu.SemaphoreType.DMA((len(cfg["wd_rows"]),)),
        ],
        compiler_params=pltpu.CompilerParams(vmem_limit_bytes=64 * 1024 * 1024,
                                             disable_bounds_checks=True,
                                             disable_semaphore_checks=True),
    )(A_x.reshape(1, D), kT, vT, A_wq, A_wo, B_w_r.reshape(D // 128, 128), B_w_gate, B_w_up, B_w_down)
    return out.reshape(B, Sq, D)


@jax.jit
def pallas_sequential_preLN__sliding_block_cached__moe_arch_mod__decode_kernel(
    A_x: jax.Array,
    A_k_cache: jax.Array,
    A_v_cache: jax.Array,
    A_wq: jax.Array,
    A_wo: jax.Array,
    B_x: jax.Array,
    B_w_r: jax.Array,
    B_w_gate: jax.Array,
    B_w_up: jax.Array,
    B_w_down: jax.Array,
):
    return _forward(A_x, A_k_cache, A_v_cache, A_wq, A_wo, B_w_r, B_w_gate, B_w_up, B_w_down, _CFG)
```

```python
import functools

import jax
import jax.numpy as jnp
import jax.experimental.pallas as pl
import jax.experimental.pallas.tpu as pltpu

_EPS = 1e-5

_CFG = dict(
    kv_blk=(96, 128),
    wq_blk=(80, 128),
    wo_blk=(32, 640),
    wgu_blk=(160, 128),
    wd_blk=(32, 640),
    wd_rows=(512, 512, 256, 128, 128),
    wd_asg=("alt", "alt", "t1", "t1", "t1"),
)


def _layernorm(x):
    m = jnp.mean(x, axis=-1, keepdims=True)
    xc = x - m
    v = jnp.mean(xc * xc, axis=-1, keepdims=True)
    return xc / jnp.sqrt(v + _EPS)


def _blocks(src, dst, sem, blk, asg="alt"):
    rows, cols = dst.shape
    br, bc = blk
    assert rows % br == 0 and cols % bc == 0, (dst.shape, blk)
    out = []
    for c in range(cols // bc):
        for r in range(rows // br):
            idx = (pl.ds(r * br, br), pl.ds(c * bc, bc))
            thread = {"alt": len(out) % 2, "t1": 1}[asg]
            out.append((src.at[idx], dst.at[idx], sem, thread))
    return out


def _merge(main, extra):
    out, k = [], 0
    n, m = len(main), len(extra)
    for i, d in enumerate(main):
        out.append(d)
        while k < m and (i + 1) * (m + 1) >= (k + 1) * n:
            out.append(extra[k])
            k += 1
    out.extend(extra[k:])
    return out


def _issue(descs):
    for src, dst, sem, thread in descs:
        pltpu.make_async_copy(src, dst, sem).start(priority=thread)


def _wait_all(sem, *dsts):
    for dst in dsts:
        pltpu.make_async_copy(dst, dst, sem).wait()


def _kernel(x_hbm, k_hbm, v_hbm, wq_hbm, wo_hbm, wr_hbm, wg_hbm, wu_hbm, wd_hbm,
            o_ref,
            x_buf, wr_buf, wq_buf, wo_buf, wg_buf, wu_buf, wd_buf, k_buf, v_buf,
            sem_misc, sem_k, sem_v, sem_wd,
            *, H, Dh, W, Sk, D, F, cfg):
    f32, bf16 = jnp.float32, jnp.bfloat16
    wd_rows = cfg["wd_rows"]
    assert sum(wd_rows) == F
    wd_off = [sum(wd_rows[:i]) for i in range(len(wd_rows))]
    n_pairs = H // 2
    win = pl.ds(Sk - W, W)

    def k_descs(h, slot, wq_slot=None):
        sem = sem_k.at[slot]
        kd = _blocks(k_hbm.at[h, :, win], k_buf.at[slot], sem, cfg["kv_blk"])
        if wq_slot is None:
            return kd
        cols = pl.ds(pl.multiple_of(h * Dh, 2 * Dh), 2 * Dh)
        return _merge(kd, _blocks(wq_hbm.at[:, cols], wq_buf.at[wq_slot], sem, cfg["wq_blk"]))

    def v_descs(h, slot):
        sem = sem_v.at[slot]
        vd = _blocks(v_hbm.at[h, :, win], v_buf.at[slot], sem, cfg["kv_blk"])
        rows = pl.ds(pl.multiple_of(h * Dh, Dh), Dh)
        return _merge(vd, _blocks(wo_hbm.at[rows, :], wo_buf.at[slot], sem, cfg["wo_blk"]))

    wg_descs = _blocks(wg_hbm, wg_buf, sem_misc.at[2], cfg["wgu_blk"])
    wu_descs = _blocks(wu_hbm, wu_buf, sem_misc.at[3], cfg["wgu_blk"])
    wd_descs = []
    for c, (o, n) in enumerate(zip(wd_off, wd_rows)):
        rows = pl.ds(o, n)
        wd_descs += _blocks(wd_hbm.at[rows, :], wd_buf.at[rows, :], sem_wd.at[c], cfg["wd_blk"], cfg["wd_asg"][c])

    x_copy = pltpu.make_async_copy(x_hbm, x_buf, sem_misc.at[0])
    wr_copy = pltpu.make_async_copy(wr_hbm, wr_buf, sem_misc.at[1])

    x_copy.start()
    wr_copy.start()
    _issue(k_descs(0, 0, 0))
    x_copy.wait()
    x = x_buf[...].astype(f32)
    xn = jnp.broadcast_to(_layernorm(x), (8, D)).astype(bf16)
    _issue(v_descs(0, 0))
    _issue(k_descs(1, 1))
    _issue(v_descs(1, 1))

    scale = Dh ** -0.5

    def head(q, slot, acc, after_qk, after_pv):
        s = jnp.dot(q, k_buf[slot], preferred_element_type=f32) * scale
        after_qk()
        m = jnp.max(s, axis=-1, keepdims=True)
        p = jnp.exp(s - m)
        l = jnp.sum(p, axis=-1, keepdims=True)
        _wait_all(sem_v.at[slot], v_buf.at[slot], wo_buf.at[slot])
        o = jax.lax.dot_general(p.astype(bf16), v_buf[slot], (((1,), (1,)), ((), ())),
                                preferred_element_type=f32)
        o = (o / l).astype(bf16)
        acc = acc + jnp.dot(o, wo_buf[slot], preferred_element_type=f32)
        after_pv()
        return acc

    def pair(j, acc, last):
        wslot = j % 2
        _wait_all(sem_k.at[0], k_buf.at[0], wq_buf.at[wslot])
        q2 = jnp.dot(xn, wq_buf[wslot], preferred_element_type=f32)
        qa = q2[:, :Dh].astype(bf16)
        qb = q2[:, Dh:].astype(bf16)
        nxt = 2 * j + 2
        nop = lambda: None
        if not last:
            acc = head(qa, 0, acc, lambda: _issue(k_descs(nxt, 0, 1 - wslot)), lambda: _issue(v_descs(nxt, 0)))
            _wait_all(sem_k.at[1], k_buf.at[1])
            acc = head(qb, 1, acc, lambda: _issue(k_descs(nxt + 1, 1)), lambda: _issue(v_descs(nxt + 1, 1)))
        else:
            acc = head(qa, 0, acc, lambda: _issue(wg_descs), nop)
            _wait_all(sem_k.at[1], k_buf.at[1])
            acc = head(qb, 1, acc, lambda: _issue(wu_descs), nop)
        return acc

    acc = jax.lax.fori_loop(0, n_pairs - 1, lambda j, a: pair(j, a, False), jnp.zeros((8, D), f32))
    attn = pair(n_pairs - 1, acc, True)

    hres = x + attn
    hn = _layernorm(hres)
    hn_b = hn.astype(bf16)
    wr_copy.wait()
    wr = wr_buf[...].astype(f32)
    r = jnp.zeros((8, 1), f32)
    for i in range(D // 128):
        r = r + jnp.sum(hn[:, i * 128:(i + 1) * 128] * wr[i:i + 1, :], axis=-1, keepdims=True)
    gate = jax.nn.sigmoid(r)
    base = hres + hn
    _issue(wd_descs)
    _wait_all(sem_misc.at[2], wg_buf)
    g = jnp.dot(hn_b, wg_buf[...], preferred_element_type=f32)
    g = g * jax.nn.sigmoid(g)
    _wait_all(sem_misc.at[3], wu_buf)
    u = jnp.dot(hn_b, wu_buf[...], preferred_element_type=f32)
    a = (g * u).astype(bf16)
    y = jnp.zeros((8, D), f32)
    for c, (o, n) in enumerate(zip(wd_off, wd_rows)):
        rows = pl.ds(o, n)
        _wait_all(sem_wd.at[c], wd_buf.at[rows, :])
        y = y + jnp.dot(a[:, o:o + n], wd_buf[rows, :], preferred_element_type=f32)
    out = base + y * gate
    o_ref[...] = out[0:1, :].astype(o_ref.dtype)


def _forward(A_x, A_k_cache, A_v_cache, A_wq, A_wo, B_w_r, B_w_gate, B_w_up, B_w_down, cfg):
    B, Sq, D = A_x.shape
    _, H, Sk, Dh = A_k_cache.shape
    F = B_w_gate.shape[1]
    W = min(4096, max(256, Sk // 4))
    assert B == 1 and Sq == 1 and A_wq.shape == (D, H * Dh) and H % 2 == 0 and H >= 4
    bf16 = jnp.bfloat16

    kT = jnp.swapaxes(A_k_cache, 2, 3).reshape(H, Dh, Sk)
    vT = jnp.swapaxes(A_v_cache, 2, 3).reshape(H, Dh, Sk)

    any_spec = pl.BlockSpec(memory_space=pl.ANY)
    out = pl.pallas_call(
        functools.partial(_kernel, H=H, Dh=Dh, W=W, Sk=Sk, D=D, F=F, cfg=cfg),
        out_shape=jax.ShapeDtypeStruct((1, D), bf16),
        in_specs=[any_spec] * 9,
        out_specs=pl.BlockSpec(memory_space=pltpu.VMEM),
        scratch_shapes=[
            pltpu.VMEM((1, D), bf16),
            pltpu.VMEM((D // 128, 128), bf16),
            pltpu.VMEM((2, D, 2 * Dh), bf16),
            pltpu.VMEM((2, Dh, D), bf16),
            pltpu.VMEM((D, F), bf16),
            pltpu.VMEM((D, F), bf16),
            pltpu.VMEM((F, D), bf16),
            pltpu.VMEM((2, Dh, W), bf16),
            pltpu.VMEM((2, Dh, W), bf16),
            pltpu.SemaphoreType.DMA((4,)),
            pltpu.SemaphoreType.DMA((2,)),
            pltpu.SemaphoreType.DMA((2,)),
            pltpu.SemaphoreType.DMA((len(cfg["wd_rows"]),)),
        ],
        compiler_params=pltpu.CompilerParams(vmem_limit_bytes=64 * 1024 * 1024,
                                             disable_bounds_checks=True,
                                             disable_semaphore_checks=True),
    )(A_x.reshape(1, D), kT, vT, A_wq, A_wo, B_w_r.reshape(D // 128, 128), B_w_gate, B_w_up, B_w_down)
    return out.reshape(B, Sq, D)


@jax.jit
def pallas_sequential_preLN__sliding_block_cached__moe_arch_mod__decode_kernel(
    A_x: jax.Array,
    A_k_cache: jax.Array,
    A_v_cache: jax.Array,
    A_wq: jax.Array,
    A_wo: jax.Array,
    B_x: jax.Array,
    B_w_r: jax.Array,
    B_w_gate: jax.Array,
    B_w_up: jax.Array,
    B_w_down: jax.Array,
):
    return _forward(A_x, A_k_cache, A_v_cache, A_wq, A_wo, B_w_r, B_w_gate, B_w_up, B_w_down, _CFG)
```
